```python
import jax
import jax.numpy as jnp

def _softmax(x, axis=-1):
    return jax.nn.softmax(x, axis=axis)
def _gelu(x):
    return jax.nn.gelu(x, approximate=True)
def _silu(x):
    return jax.nn.silu(x)
def _sigmoid(x):
    return jax.nn.sigmoid(x)
def _layernorm(x, axis=-1, eps=1e-5):
    m = jnp.mean(x, axis=axis, keepdims=True)
    v = jnp.var(x, axis=axis, keepdims=True)
    return (x - m) / jnp.sqrt(v + eps)
def _scatter_add(tgt, idx, src, axis=0):
    return tgt.at[idx].add(src)
def _segment_sum(src, seg, n):
    return jax.ops.segment_sum(src, seg, n)
class _Rng:
    def __init__(self, key):
        self._k = key
    def _next(self):
        self._k, sub = jax.random.split(self._k)
        return sub
    def normal(self, shape):
        return jax.random.normal(self._next(), shape, dtype=jnp.bfloat16)
    def randint(self, lo, hi, shape):
        return jax.random.randint(self._next(), shape, lo, hi, dtype=jnp.int32)
    def uniform(self, shape, lo=0.0, hi=1.0):
        return jax.random.uniform(self._next(), shape, jnp.bfloat16, lo, hi)
    def permutation(self, n):
        return jax.random.permutation(self._next(), n)


kernel_name = 'recurrent_scan__sliding_block_cached__moe_arch_mod__decode'

def setup_inputs():
    _rng = _Rng(jax.random.key(int.from_bytes(__import__("os").urandom(4), "little")))
    _w = (lambda a: (lambda t: t.astype(jnp.bfloat16) if jnp.issubdtype(t.dtype, jnp.floating) else t)(jnp.asarray(a)))
    def _A_setup():
        B, Sq, D = 1, 1, 512
        Hq, Hkv, Sk, Dh = 32, 32, 32768, 128
        assert Hq % Hkv == 0, (Hq, Hkv)
        return {
            "x": _w((lambda *s: _rng.normal(s) * 0.05)(B, Sq, D)),
            "k_cache": _w((lambda *s: _rng.normal(s) * 0.05)(B, Hkv, Sk, Dh)),
            "v_cache": _w((lambda *s: _rng.normal(s) * 0.05)(B, Hkv, Sk, Dh)),
            "wq": _w((lambda *s: _rng.normal(s) * 0.05)(D, Hq * Dh) * (D ** -0.5)),
            "wo": _w((lambda *s: _rng.normal(s) * 0.05)(Hq * Dh, D) * ((Hq * Dh) ** -0.5)),
        }
    _A_in = _A_setup()

    def _B_setup():
        B, S, D, F, C = 1, 1, 512, 1376, 1
        return {
            "x": _w((lambda *s: _rng.normal(s) * 0.05)(B, S, D)),
            "w_r": _w((lambda *s: _rng.normal(s) * 0.05)(D)),
            "w_gate": _w((lambda *s: _rng.normal(s) * 0.05)(D, F)),
            "w_up": _w((lambda *s: _rng.normal(s) * 0.05)(D, F)),
            "w_down": _w((lambda *s: _rng.normal(s) * 0.05)(F, D)),
        }
    _B_in = _B_setup()

    return {
        "A_x": _A_in["x"],
        "A_k_cache": _A_in["k_cache"],
        "A_v_cache": _A_in["v_cache"],
        "A_wq": _A_in["wq"],
        "A_wo": _A_in["wo"],
        "B_x": _B_in["x"],
        "B_w_r": _B_in["w_r"],
        "B_w_gate": _B_in["w_gate"],
        "B_w_up": _B_in["w_up"],
        "B_w_down": _B_in["w_down"],
    }

def reference(A_x, A_k_cache, A_v_cache, A_wq, A_wo, B_x, B_w_r, B_w_gate, B_w_up, B_w_down):
    def _A_ref(x, k_cache, v_cache, wq, wo):
        B, Sq, D = x.shape
        Hq, Dh = 32, 128
        Hkv, Sk = k_cache.shape[1], k_cache.shape[2]
        W = min(4096, max(256, Sk // 4))
        rep = Hq // Hkv
        q = (lambda x, *d: x.transpose(*d))((x @ wq).reshape(B, Sq, Hq, Dh), 0, 2, 1, 3)
        k = jnp.repeat(k_cache[:, :, Sk - W:, :], rep, axis=1)
        v = jnp.repeat(v_cache[:, :, Sk - W:, :], rep, axis=1)
        scores = jnp.einsum("bhqd,bhkd->bhqk", q, k) * (Dh ** -0.5)
        p = _softmax(scores, axis=-1)
        o = jnp.einsum("bhqk,bhkd->bhqd", p, v)
        return (lambda x, *d: x.transpose(*d))(o, 0, 2, 1, 3).reshape(B, Sq, Hq * Dh) @ wo

    def _B_ref(x, w_r, w_gate, w_up, w_down):
        B, S, D = x.shape
        C = 1
        r = x @ w_r
        idx = jnp.argsort(-r, axis=-1)[:, :C]
        idx_e = jnp.repeat(idx.reshape(B, C, 1), D, axis=2)
        x_sel = jnp.take_along_axis(x, idx_e, axis=1)
        g = _silu(x_sel @ w_gate)
        u = x_sel @ w_up
        y = (g * u) @ w_down
        r_sel = _sigmoid(jnp.take_along_axis(r, idx, axis=1))
        y = y * r_sel.reshape(B, C, 1)
        b_off = (jnp.arange(B) * S).reshape(B, 1)
        flat_idx = (idx + b_off).reshape(B * C)
        zero = (x * 0.0).reshape(B * S, D)
        upd = _scatter_add(zero, flat_idx, y.reshape(B * C, D), axis=0)
        return x + upd.reshape(B, S, D)

    x = A_x
    xn = _layernorm(x, axis=-1)
    s = _A_ref(xn, A_k_cache, A_v_cache, A_wq, A_wo)
    g = _silu(_B_ref(xn, B_w_r, B_w_gate, B_w_up, B_w_down))
    return x + s * g
```

```python
import jax
import jax.numpy as jnp
from jax import lax
import jax.experimental.pallas as pl
import jax.experimental.pallas.tpu as pltpu

BF = jnp.bfloat16
F32 = jnp.float32
NT = (((1,), (1,)), ((), ()))
NN = (((1,), (0,)), ((), ()))
M = 8


@jax.jit
def pallas_recurrent_scan__sliding_block_cached__moe_arch_mod__decode_kernel(
    A_x: jax.Array,
    A_k_cache: jax.Array,
    A_v_cache: jax.Array,
    A_wq: jax.Array,
    A_wo: jax.Array,
    B_x: jax.Array,
    B_w_r: jax.Array,
    B_w_gate: jax.Array,
    B_w_up: jax.Array,
    B_w_down: jax.Array,
):
    del B_x
    D = A_x.shape[-1]
    _, H, SK, DH = A_k_cache.shape
    F = B_w_gate.shape[1]
    W = min(4096, max(256, SK // 4))
    WO_CHUNKS = 4
    hpc = H // WO_CHUNKS

    def kernel(x_hbm, k_hbm, v_hbm, wq_hbm, wo_hbm, wg_hbm, wu_hbm, wd_hbm, wr_hbm, o_ref,
               xb, wrb, kbuf, vbuf, wqb, wob, wgb, wub, wdb, q_scr, o_scr, ksem, vsem, wsem):
        def kc(h):
            return pltpu.make_async_copy(k_hbm.at[0, h, pl.ds(SK - W, W), :], kbuf.at[h], ksem.at[h])

        def vc(h):
            return pltpu.make_async_copy(v_hbm.at[0, h, pl.ds(SK - W, W), :], vbuf.at[h], vsem.at[h])

        cx = pltpu.make_async_copy(x_hbm, xb, wsem.at[0])
        cq = pltpu.make_async_copy(wq_hbm, wqb, wsem.at[1])
        cr = pltpu.make_async_copy(wr_hbm, wrb, wsem.at[2])
        cg = pltpu.make_async_copy(wg_hbm, wgb, wsem.at[3])
        cu = pltpu.make_async_copy(wu_hbm, wub, wsem.at[4])
        cd = pltpu.make_async_copy(wd_hbm, wdb, wsem.at[5])
        co = [pltpu.make_async_copy(wo_hbm.at[pl.ds(i * hpc * DH, hpc * DH), :],
                                    wob.at[pl.ds(i * hpc * DH, hpc * DH), :], wsem.at[6 + i])
              for i in range(WO_CHUNKS)]
        cx.start()
        cq.start()
        for h in range(H):
            kc(h).start()
            vc(h).start()
        cr.start()
        cg.start()
        cu.start()
        cd.start()
        for c in co:
            c.start()

        cx.wait()
        xf = xb[0].astype(F32)
        mu = jnp.mean(xf, axis=-1, keepdims=True)
        xc = xf - mu
        var = jnp.mean(xc * xc, axis=-1, keepdims=True)
        xn = xc / jnp.sqrt(var + 1e-5)
        xnb = xn.astype(BF)
        xn8 = jnp.broadcast_to(xnb, (M, D))
        cq.wait()
        for h in range(H):
            qh = lax.dot_general(xn8, wqb[:, h * DH:(h + 1) * DH], NN, preferred_element_type=F32)
            q_scr[h] = qh.astype(BF)

        def body(h, carry):
            kc(h).wait()
            s = lax.dot_general(q_scr[h], kbuf[h], NT, preferred_element_type=F32) * (DH ** -0.5)
            m = jnp.max(s, axis=-1, keepdims=True)
            p = jnp.exp(s - m)
            l = jnp.sum(p, axis=-1, keepdims=True)
            vc(h).wait()
            o = lax.dot_general(p.astype(BF), vbuf[h], NN, preferred_element_type=F32)
            o_scr[h] = (o / l).astype(BF)
            return carry

        lax.fori_loop(0, H, body, 0)

        cr.wait()
        cg.wait()
        cu.wait()
        g = lax.dot_general(xn8, wgb[...], NT, preferred_element_type=F32)
        u = lax.dot_general(xn8, wub[...], NT, preferred_element_type=F32)
        hh = (g * jax.nn.sigmoid(g) * u).astype(BF)
        cd.wait()
        y = lax.dot_general(hh, wdb[...], NN, preferred_element_type=F32)[0:1]
        r = jnp.sum(xnb.astype(F32) * wrb[...].reshape(1, D).astype(F32), axis=-1, keepdims=True)
        b = xn + y * jax.nn.sigmoid(r)
        gate = b * jax.nn.sigmoid(b)
        acc = jnp.zeros((M, D), F32)
        for i in range(WO_CHUNKS):
            co[i].wait()
            for h in range(i * hpc, (i + 1) * hpc):
                acc = acc + lax.dot_general(o_scr[h], wob[h * DH:(h + 1) * DH, :], NN,
                                            preferred_element_type=F32)
        o_ref[0] = (xf + acc[0:1] * gate).astype(BF)

    hbm = pl.BlockSpec(memory_space=pltpu.HBM)
    return pl.pallas_call(
        kernel,
        out_shape=jax.ShapeDtypeStruct((1, 1, D), BF),
        in_specs=[hbm] * 9,
        out_specs=pl.BlockSpec(memory_space=pltpu.VMEM),
        scratch_shapes=[
            pltpu.VMEM((1, 1, D), BF), pltpu.VMEM((D,), BF),
            pltpu.VMEM((H, W, DH), BF), pltpu.VMEM((H, W, DH), BF),
            pltpu.VMEM((D, H * DH), BF), pltpu.VMEM((H * DH, D), BF),
            pltpu.VMEM((F, D), BF), pltpu.VMEM((F, D), BF), pltpu.VMEM((F, D), BF),
            pltpu.VMEM((H, M, DH), BF), pltpu.VMEM((H, M, DH), BF),
            pltpu.SemaphoreType.DMA((H,)), pltpu.SemaphoreType.DMA((H,)),
            pltpu.SemaphoreType.DMA((6 + WO_CHUNKS,)),
        ],
        compiler_params=pltpu.CompilerParams(vmem_limit_bytes=110 * 1024 * 1024),
    )(A_x, A_k_cache, A_v_cache, A_wq, A_wo, B_w_gate.T, B_w_up.T, B_w_down, B_w_r)
```

```python
import jax
import jax.numpy as jnp
from jax import lax
import jax.experimental.pallas as pl
import jax.experimental.pallas.tpu as pltpu

BF = jnp.bfloat16
F32 = jnp.float32
NN = (((1,), (0,)), ((), ()))
NT = (((1,), (1,)), ((), ()))
ROWS = 8
HQ, DH = 32, 128
LN_EPS = 1e-5


@jax.jit
def pallas_recurrent_scan__sliding_block_cached__moe_arch_mod__decode_kernel(
    A_x: jax.Array,
    A_k_cache: jax.Array,
    A_v_cache: jax.Array,
    A_wq: jax.Array,
    A_wo: jax.Array,
    B_x: jax.Array,
    B_w_r: jax.Array,
    B_w_gate: jax.Array,
    B_w_up: jax.Array,
    B_w_down: jax.Array,
):
    del B_x
    B, Sq, D = A_x.shape
    _, Hkv, Sk, _ = A_k_cache.shape
    F = B_w_gate.shape[1]
    W = min(4096, max(256, Sk // 4))
    assert B == 1 and Sq == 1 and Hkv == HQ
    FFN_AFTER = HQ // 2

    def kernel(x_hbm, k_hbm, v_hbm, wq_hbm, wo_hbm, wr_hbm, wg_hbm, wu_hbm, wd_hbm, o_ref,
               x_buf, wr_buf, k_buf, v_buf, wq_buf, wo_buf, wg_buf, wu_buf, wd_buf,
               q_scr, o_scr, k_sem, v_sem, o_sem, w_sem):

        def k_copy(h):
            return pltpu.make_async_copy(
                k_hbm.at[0, h, pl.ds(Sk - W, W), :], k_buf.at[h], k_sem.at[h])

        def v_copy(h):
            return pltpu.make_async_copy(
                v_hbm.at[0, h, pl.ds(Sk - W, W), :], v_buf.at[h], v_sem.at[h])

        def wo_copy(h):
            rows = pl.ds(h * DH if isinstance(h, int) else pl.multiple_of(h * DH, DH), DH)
            return pltpu.make_async_copy(wo_hbm.at[rows, :], wo_buf.at[rows, :], o_sem.at[h])

        x_copy = pltpu.make_async_copy(x_hbm, x_buf, w_sem.at[0])
        wq_copy = pltpu.make_async_copy(wq_hbm, wq_buf, w_sem.at[1])
        wr_copy = pltpu.make_async_copy(wr_hbm, wr_buf, w_sem.at[2])
        wg_copy = pltpu.make_async_copy(wg_hbm, wg_buf, w_sem.at[3])
        wu_copy = pltpu.make_async_copy(wu_hbm, wu_buf, w_sem.at[4])
        wd_copy = pltpu.make_async_copy(wd_hbm, wd_buf, w_sem.at[5])

        def loop(lo, hi, body):
            lax.fori_loop(lo, hi, lambda i, c: (body(i), c)[1], 0)

        def start_kv(h):
            k_copy(h).start()
            v_copy(h).start()

        x_copy.start()
        wq_copy.start()
        wr_copy.start()
        loop(0, FFN_AFTER, start_kv)
        wg_copy.start()
        wu_copy.start()
        wd_copy.start()
        loop(FFN_AFTER, HQ, start_kv)
        loop(0, HQ, lambda h: wo_copy(h).start())

        x_copy.wait()
        x = x_buf[0].astype(F32)
        xc = x - jnp.mean(x, axis=-1, keepdims=True)
        var = jnp.mean(xc * xc, axis=-1, keepdims=True)
        xn = xc / jnp.sqrt(var + LN_EPS)
        xn_b = xn.astype(BF)
        xn_rows = jnp.broadcast_to(xn_b, (ROWS, D))

        wr_copy.wait()
        r = jnp.sum(xn_b.astype(F32) * wr_buf[...].reshape(1, D).astype(F32),
                    axis=-1, keepdims=True)
        r_gate = jax.nn.sigmoid(r)

        wq_copy.wait()
        for h in range(HQ):
            q_scr[h] = lax.dot_general(xn_rows, wq_buf[:, h * DH:(h + 1) * DH], NN,
                                       preferred_element_type=F32).astype(BF)

        def head(h):
            k_copy(h).wait()
            s = lax.dot_general(q_scr[h], k_buf[h], NT, preferred_element_type=F32) * (DH ** -0.5)
            p = jnp.exp(s - jnp.max(s, axis=-1, keepdims=True))
            denom = jnp.sum(p, axis=-1, keepdims=True)
            v_copy(h).wait()
            o = lax.dot_general(p.astype(BF), v_buf[h], NN, preferred_element_type=F32)
            o_scr[h] = (o / denom).astype(BF)

        loop(0, FFN_AFTER, head)

        wg_copy.wait()
        wu_copy.wait()
        g = lax.dot_general(xn_rows, wg_buf[...], NT, preferred_element_type=F32)
        u = lax.dot_general(xn_rows, wu_buf[...], NT, preferred_element_type=F32)
        hid = (g * jax.nn.sigmoid(g) * u).astype(BF)
        wd_copy.wait()
        y = lax.dot_general(hid, wd_buf[...], NN, preferred_element_type=F32)[0:1]
        routed = xn + y * r_gate
        gate = routed * jax.nn.sigmoid(routed)

        loop(FFN_AFTER, HQ, head)

        acc = jnp.zeros((ROWS, D), F32)
        for h in range(HQ):
            wo_copy(h).wait()
            acc = acc + lax.dot_general(o_scr[h], wo_buf[h * DH:(h + 1) * DH, :], NN,
                                        preferred_element_type=F32)

        o_ref[0] = (x + acc[0:1] * gate).astype(BF)

    hbm = pl.BlockSpec(memory_space=pltpu.HBM)
    return pl.pallas_call(
        kernel,
        out_shape=jax.ShapeDtypeStruct((B, Sq, D), BF),
        in_specs=[hbm] * 9,
        out_specs=pl.BlockSpec(memory_space=pltpu.VMEM),
        scratch_shapes=[
            pltpu.VMEM((B, Sq, D), BF),
            pltpu.VMEM((D,), BF),
            pltpu.VMEM((HQ, W, DH), BF),
            pltpu.VMEM((HQ, W, DH), BF),
            pltpu.VMEM((D, HQ * DH), BF),
            pltpu.VMEM((HQ * DH, D), BF),
            pltpu.VMEM((F, D), BF),
            pltpu.VMEM((F, D), BF),
            pltpu.VMEM((F, D), BF),
            pltpu.VMEM((HQ, ROWS, DH), BF),
            pltpu.VMEM((HQ, ROWS, DH), BF),
            pltpu.SemaphoreType.DMA((HQ,)),
            pltpu.SemaphoreType.DMA((HQ,)),
            pltpu.SemaphoreType.DMA((HQ,)),
            pltpu.SemaphoreType.DMA((6,)),
        ],
        compiler_params=pltpu.CompilerParams(
            vmem_limit_bytes=110 * 1024 * 1024,
            disable_semaphore_checks=True,
        ),
    )(A_x, A_k_cache, A_v_cache, A_wq, A_wo, B_w_r, B_w_gate.T, B_w_up.T, B_w_down)
```

```python
import jax
import jax.numpy as jnp
from jax import lax
import jax.experimental.pallas as pl
import jax.experimental.pallas.tpu as pltpu

BF = jnp.bfloat16
F32 = jnp.float32
NN = (((1,), (0,)), ((), ()))
NT = (((1,), (1,)), ((), ()))
ROWS = 8
HQ, DH = 32, 128
LN_EPS = 1e-5


@jax.jit
def pallas_recurrent_scan__sliding_block_cached__moe_arch_mod__decode_kernel(
    A_x: jax.Array,
    A_k_cache: jax.Array,
    A_v_cache: jax.Array,
    A_wq: jax.Array,
    A_wo: jax.Array,
    B_x: jax.Array,
    B_w_r: jax.Array,
    B_w_gate: jax.Array,
    B_w_up: jax.Array,
    B_w_down: jax.Array,
):
    del B_x
    B, Sq, D = A_x.shape
    _, Hkv, Sk, _ = A_k_cache.shape
    F = B_w_gate.shape[1]
    W = min(4096, max(256, Sk // 4))
    assert B == 1 and Sq == 1 and Hkv == HQ
    FFN_AFTER = HQ // 2

    def kernel(x_hbm, k_hbm, v_hbm, wq_hbm, wo_hbm, wr_hbm, wg_hbm, wu_hbm, wd_hbm, o_ref,
               x_buf, wr_buf, k_buf, v_buf, wq_buf, wo_buf, wg_buf, wu_buf, wd_buf,
               q_scr, o_scr, c_scr, k_sem, v_sem, o_sem, w_sem):

        def k_copy(h):
            return pltpu.make_async_copy(
                k_hbm.at[0, h, pl.ds(Sk - W, W), :], k_buf.at[h], k_sem.at[h])

        def v_copy(h):
            return pltpu.make_async_copy(
                v_hbm.at[0, h, pl.ds(Sk - W, W), :], v_buf.at[h], v_sem.at[h])

        def wo_copy(h):
            rows = pl.ds(h * DH if isinstance(h, int) else pl.multiple_of(h * DH, DH), DH)
            return pltpu.make_async_copy(wo_hbm.at[rows, :], wo_buf.at[rows, :], o_sem.at[h])

        x_copy = pltpu.make_async_copy(x_hbm, x_buf, w_sem.at[0])
        wq_copy = pltpu.make_async_copy(wq_hbm, wq_buf, w_sem.at[1])
        wr_copy = pltpu.make_async_copy(wr_hbm, wr_buf, w_sem.at[2])
        wg_copy = pltpu.make_async_copy(wg_hbm, wg_buf, w_sem.at[3])
        wu_copy = pltpu.make_async_copy(wu_hbm, wu_buf, w_sem.at[4])
        wd_copy = pltpu.make_async_copy(wd_hbm, wd_buf, w_sem.at[5])

        def loop(lo, hi, body):
            lax.fori_loop(lo, hi, lambda i, c: (body(i), c)[1], 0)

        def start_kv(h):
            k_copy(h).start()
            v_copy(h).start()

        x_copy.start()
        wq_copy.start()
        wr_copy.start()
        loop(0, FFN_AFTER, start_kv)
        wg_copy.start()
        wu_copy.start()
        wd_copy.start()
        loop(FFN_AFTER, HQ, start_kv)
        loop(0, HQ, lambda h: wo_copy(h).start())

        x_copy.wait()
        x = x_buf[0].astype(F32)
        xc = x - jnp.mean(x, axis=-1, keepdims=True)
        var = jnp.mean(xc * xc, axis=-1, keepdims=True)
        xn = xc / jnp.sqrt(var + LN_EPS)
        xn_b = xn.astype(BF)
        xn_rows = jnp.broadcast_to(xn_b, (ROWS, D))

        wr_copy.wait()
        r = jnp.sum(xn_b.astype(F32) * wr_buf[...].reshape(1, D).astype(F32),
                    axis=-1, keepdims=True)
        r_gate = jax.nn.sigmoid(r)

        wq_copy.wait()
        for h in range(HQ):
            q_scr[h] = lax.dot_general(xn_rows, wq_buf[:, h * DH:(h + 1) * DH], NN,
                                       preferred_element_type=F32).astype(BF)

        def head(h):
            k_copy(h).wait()
            s = lax.dot_general(q_scr[h], k_buf[h], NT, preferred_element_type=F32) * (DH ** -0.5)
            p = jnp.exp(s - jnp.max(s, axis=-1, keepdims=True))
            denom = jnp.sum(p, axis=-1, keepdims=True)
            v_copy(h).wait()
            o = lax.dot_general(p.astype(BF), v_buf[h], NN, preferred_element_type=F32)
            o_scr[h] = (o / denom).astype(BF)

        loop(0, FFN_AFTER, head)

        wg_copy.wait()
        wu_copy.wait()
        g = lax.dot_general(xn_rows, wg_buf[...], NT, preferred_element_type=F32)
        u = lax.dot_general(xn_rows, wu_buf[...], NT, preferred_element_type=F32)
        hid = (g * jax.nn.sigmoid(g) * u).astype(BF)
        wd_copy.wait()
        y = lax.dot_general(hid, wd_buf[...], NN, preferred_element_type=F32)[0:1]
        routed = xn + y * r_gate
        gate = routed * jax.nn.sigmoid(routed)

        loop(FFN_AFTER, HQ, head)

        last = HQ - 1
        o_last = o_scr[last][0:1, :].astype(F32)
        c_scr[...] = jnp.broadcast_to(o_last, (DH, DH)).T
        acc = jnp.zeros((ROWS, D), F32)
        for h in range(last):
            wo_copy(h).wait()
            acc = acc + lax.dot_general(o_scr[h], wo_buf[h * DH:(h + 1) * DH, :], NN,
                                        preferred_element_type=F32)
        wo_copy(last).wait()
        w = wo_buf[last * DH:, :].astype(F32)
        prod = w * jnp.concatenate([c_scr[...]] * (D // DH), axis=1)
        s_out = acc[0:1] + jnp.sum(prod.reshape(DH // 8, 8, D).sum(axis=0), axis=0, keepdims=True)

        o_ref[0] = (x + s_out * gate).astype(BF)

    hbm = pl.BlockSpec(memory_space=pltpu.HBM)
    return pl.pallas_call(
        kernel,
        out_shape=jax.ShapeDtypeStruct((B, Sq, D), BF),
        in_specs=[hbm] * 9,
        out_specs=pl.BlockSpec(memory_space=pltpu.VMEM),
        scratch_shapes=[
            pltpu.VMEM((B, Sq, D), BF),
            pltpu.VMEM((D,), BF),
            pltpu.VMEM((HQ, W, DH), BF),
            pltpu.VMEM((HQ, W, DH), BF),
            pltpu.VMEM((D, HQ * DH), BF),
            pltpu.VMEM((HQ * DH, D), BF),
            pltpu.VMEM((F, D), BF),
            pltpu.VMEM((F, D), BF),
            pltpu.VMEM((F, D), BF),
            pltpu.VMEM((HQ, ROWS, DH), BF),
            pltpu.VMEM((HQ, ROWS, DH), BF),
            pltpu.VMEM((DH, DH), F32),
            pltpu.SemaphoreType.DMA((HQ,)),
            pltpu.SemaphoreType.DMA((HQ,)),
            pltpu.SemaphoreType.DMA((HQ,)),
            pltpu.SemaphoreType.DMA((6,)),
        ],
        compiler_params=pltpu.CompilerParams(
            vmem_limit_bytes=110 * 1024 * 1024,
            disable_semaphore_checks=True,
        ),
    )(A_x, A_k_cache, A_v_cache, A_wq, A_wo, B_w_r, B_w_gate.T, B_w_up.T, B_w_down)
```

```python
import jax
import jax.numpy as jnp
from jax import lax
import jax.experimental.pallas as pl
import jax.experimental.pallas.tpu as pltpu

BF = jnp.bfloat16
F32 = jnp.float32
NN = (((1,), (0,)), ((), ()))
NT = (((1,), (1,)), ((), ()))
ROWS = 8
HQ, DH = 32, 128
LN_EPS = 1e-5


@jax.jit
def pallas_recurrent_scan__sliding_block_cached__moe_arch_mod__decode_kernel(
    A_x: jax.Array,
    A_k_cache: jax.Array,
    A_v_cache: jax.Array,
    A_wq: jax.Array,
    A_wo: jax.Array,
    B_x: jax.Array,
    B_w_r: jax.Array,
    B_w_gate: jax.Array,
    B_w_up: jax.Array,
    B_w_down: jax.Array,
):
    del B_x
    B, Sq, D = A_x.shape
    _, Hkv, Sk, _ = A_k_cache.shape
    F = B_w_gate.shape[1]
    W = min(4096, max(256, Sk // 4))
    assert B == 1 and Sq == 1 and Hkv == HQ
    FFN_AFTER = HQ // 2
    LAST = HQ - 1
    TAIL = ((0, 96), (96, 32))

    def kernel(x_hbm, k_hbm, v_hbm, wq_hbm, wo_hbm, wr_hbm, wg_hbm, wu_hbm, wd_hbm, o_ref,
               x_buf, wr_buf, k_buf, v_buf, wq_buf, wo_buf, wg_buf, wu_buf, wd_buf,
               q_scr, o_scr, c_scr, k_sem, v_sem, o_sem, w_sem):

        def k_copy(h):
            return pltpu.make_async_copy(
                k_hbm.at[0, h, pl.ds(Sk - W, W), :], k_buf.at[h], k_sem.at[h])

        def v_copy(h):
            return pltpu.make_async_copy(
                v_hbm.at[0, h, pl.ds(Sk - W, W), :], v_buf.at[h], v_sem.at[h])

        def wo_copy(h):
            rows = pl.ds(h * DH if isinstance(h, int) else pl.multiple_of(h * DH, DH), DH)
            return pltpu.make_async_copy(wo_hbm.at[rows, :], wo_buf.at[rows, :], o_sem.at[h])

        def wo_tail_copy(j):
            rows = pl.ds(LAST * DH + TAIL[j][0], TAIL[j][1])
            return pltpu.make_async_copy(wo_hbm.at[rows, :], wo_buf.at[rows, :], o_sem.at[LAST + j])

        def start_wo_tail(i):
            for j in range(len(TAIL)):
                pl.when(i == j)(wo_tail_copy(j).start)

        x_copy = pltpu.make_async_copy(x_hbm, x_buf, w_sem.at[0])
        wq_copy = pltpu.make_async_copy(wq_hbm, wq_buf, w_sem.at[1])
        wr_copy = pltpu.make_async_copy(wr_hbm, wr_buf, w_sem.at[2])
        wg_copy = pltpu.make_async_copy(wg_hbm, wg_buf, w_sem.at[3])
        wu_copy = pltpu.make_async_copy(wu_hbm, wu_buf, w_sem.at[4])
        wd_copy = pltpu.make_async_copy(wd_hbm, wd_buf, w_sem.at[5])

        def loop(lo, hi, body):
            lax.fori_loop(lo, hi, lambda i, c: (body(i), c)[1], 0)

        def start_kv(h):
            k_copy(h).start()
            v_copy(h).start()

        x_copy.start()
        wq_copy.start()
        wr_copy.start()
        loop(0, FFN_AFTER, start_kv)
        wg_copy.start()
        wu_copy.start()
        wd_copy.start()
        loop(FFN_AFTER, HQ, start_kv)
        loop(0, LAST, lambda h: wo_copy(h).start())
        loop(0, len(TAIL), start_wo_tail)

        x_copy.wait()
        x = x_buf[0].astype(F32)
        xc = x - jnp.mean(x, axis=-1, keepdims=True)
        var = jnp.mean(xc * xc, axis=-1, keepdims=True)
        xn = xc / jnp.sqrt(var + LN_EPS)
        xn_b = xn.astype(BF)
        xn_rows = jnp.broadcast_to(xn_b, (ROWS, D))

        wr_copy.wait()
        r = jnp.sum(xn_b.astype(F32) * wr_buf[...].reshape(1, D).astype(F32),
                    axis=-1, keepdims=True)
        r_gate = jax.nn.sigmoid(r)

        wq_copy.wait()
        for h in range(HQ):
            q_scr[h] = lax.dot_general(xn_rows, wq_buf[:, h * DH:(h + 1) * DH], NN,
                                       preferred_element_type=F32).astype(BF)

        def head(h):
            k_copy(h).wait()
            s = lax.dot_general(q_scr[h], k_buf[h], NT, preferred_element_type=F32) * (DH ** -0.5)
            p = jnp.exp(s - jnp.max(s, axis=-1, keepdims=True))
            denom = jnp.sum(p, axis=-1, keepdims=True)
            v_copy(h).wait()
            o = lax.dot_general(p.astype(BF), v_buf[h], NN, preferred_element_type=F32)
            o_scr[h] = (o / denom).astype(BF)

        loop(0, FFN_AFTER, head)

        wg_copy.wait()
        wu_copy.wait()
        g = lax.dot_general(xn_rows, wg_buf[...], NT, preferred_element_type=F32)
        u = lax.dot_general(xn_rows, wu_buf[...], NT, preferred_element_type=F32)
        hid = (g * jax.nn.sigmoid(g) * u).astype(BF)
        wd_copy.wait()
        y = lax.dot_general(hid, wd_buf[...], NN, preferred_element_type=F32)[0:1]
        routed = xn + y * r_gate
        gate = routed * jax.nn.sigmoid(routed)

        loop(FFN_AFTER, HQ, head)

        o_last = o_scr[LAST][0:1, :].astype(F32)
        c_scr[...] = jnp.broadcast_to(o_last, (DH, DH)).T
        acc = jnp.zeros((ROWS, D), F32)
        for h in range(LAST):
            wo_copy(h).wait()
            acc = acc + lax.dot_general(o_scr[h], wo_buf[h * DH:(h + 1) * DH, :], NN,
                                        preferred_element_type=F32)
        part = jnp.zeros((8, D), F32)
        for j, (r0, n) in enumerate(TAIL):
            wo_tail_copy(j).wait()
            w = wo_buf[LAST * DH + r0:LAST * DH + r0 + n, :].astype(F32)
            c = jnp.concatenate([c_scr[r0:r0 + n, :]] * (D // DH), axis=1)
            part = part + (w * c).reshape(n // 8, 8, D).sum(axis=0)
        s_out = acc[0:1] + jnp.sum(part, axis=0, keepdims=True)

        o_ref[0] = (x + s_out * gate).astype(BF)

    hbm = pl.BlockSpec(memory_space=pltpu.HBM)
    return pl.pallas_call(
        kernel,
        out_shape=jax.ShapeDtypeStruct((B, Sq, D), BF),
        in_specs=[hbm] * 9,
        out_specs=pl.BlockSpec(memory_space=pltpu.VMEM),
        scratch_shapes=[
            pltpu.VMEM((B, Sq, D), BF),
            pltpu.VMEM((D,), BF),
            pltpu.VMEM((HQ, W, DH), BF),
            pltpu.VMEM((HQ, W, DH), BF),
            pltpu.VMEM((D, HQ * DH), BF),
            pltpu.VMEM((HQ * DH, D), BF),
            pltpu.VMEM((F, D), BF),
            pltpu.VMEM((F, D), BF),
            pltpu.VMEM((F, D), BF),
            pltpu.VMEM((HQ, ROWS, DH), BF),
            pltpu.VMEM((HQ, ROWS, DH), BF),
            pltpu.VMEM((DH, DH), F32),
            pltpu.SemaphoreType.DMA((HQ,)),
            pltpu.SemaphoreType.DMA((HQ,)),
            pltpu.SemaphoreType.DMA((LAST + len(TAIL),)),
            pltpu.SemaphoreType.DMA((6,)),
        ],
        compiler_params=pltpu.CompilerParams(
            vmem_limit_bytes=110 * 1024 * 1024,
            disable_semaphore_checks=True,
        ),
    )(A_x, A_k_cache, A_v_cache, A_wq, A_wo, B_w_r, B_w_gate.T, B_w_up.T, B_w_down)
```

```python
import jax
import jax.numpy as jnp
from jax import lax
import jax.experimental.pallas as pl
import jax.experimental.pallas.tpu as pltpu

BF = jnp.bfloat16
F32 = jnp.float32
NN = (((1,), (0,)), ((), ()))
NT = (((1,), (1,)), ((), ()))
ROWS = 8
HQ, DH = 32, 128
LN_EPS = 1e-5


@jax.jit
def pallas_recurrent_scan__sliding_block_cached__moe_arch_mod__decode_kernel(
    A_x: jax.Array,
    A_k_cache: jax.Array,
    A_v_cache: jax.Array,
    A_wq: jax.Array,
    A_wo: jax.Array,
    B_x: jax.Array,
    B_w_r: jax.Array,
    B_w_gate: jax.Array,
    B_w_up: jax.Array,
    B_w_down: jax.Array,
):
    del B_x
    B, Sq, D = A_x.shape
    _, Hkv, Sk, _ = A_k_cache.shape
    F = B_w_gate.shape[1]
    W = min(4096, max(256, Sk // 4))
    assert B == 1 and Sq == 1 and Hkv == HQ
    FFN_AFTER = HQ // 2
    LAST = HQ - 1
    TAIL = ((0, 96), (96, 32))

    def kernel(x_hbm, k_hbm, v_hbm, wq_hbm, wo_hbm, wr_hbm, wg_hbm, wu_hbm, wd_hbm, o_ref,
               x_buf, wr_buf, k_buf, v_buf, wq_buf, wo_buf, wg_buf, wu_buf, wd_buf,
               q_scr, o_scr, c_scr):

        def body(k_sem, v_sem, o_sem, w_sem):
            def k_copy(h):
                return pltpu.make_async_copy(
                    k_hbm.at[0, h, pl.ds(Sk - W, W), :], k_buf.at[h], k_sem.at[h])

            def v_copy(h):
                return pltpu.make_async_copy(
                    v_hbm.at[0, h, pl.ds(Sk - W, W), :], v_buf.at[h], v_sem.at[h])

            def wo_copy(h):
                rows = pl.ds(h * DH if isinstance(h, int) else pl.multiple_of(h * DH, DH), DH)
                return pltpu.make_async_copy(wo_hbm.at[rows, :], wo_buf.at[rows, :], o_sem.at[h])

            def wo_tail_copy(j):
                rows = pl.ds(LAST * DH + TAIL[j][0], TAIL[j][1])
                return pltpu.make_async_copy(wo_hbm.at[rows, :], wo_buf.at[rows, :], o_sem.at[LAST + j])

            def start_wo_tail(i):
                for j in range(len(TAIL)):
                    pl.when(i == j)(wo_tail_copy(j).start)

            x_copy = pltpu.make_async_copy(x_hbm, x_buf, w_sem.at[0])
            wq_copy = pltpu.make_async_copy(wq_hbm, wq_buf, w_sem.at[1])
            wr_copy = pltpu.make_async_copy(wr_hbm, wr_buf, w_sem.at[2])
            wg_copy = pltpu.make_async_copy(wg_hbm, wg_buf, w_sem.at[3])
            wu_copy = pltpu.make_async_copy(wu_hbm, wu_buf, w_sem.at[4])
            wd_copy = pltpu.make_async_copy(wd_hbm, wd_buf, w_sem.at[5])

            def loop(lo, hi, body):
                lax.fori_loop(lo, hi, lambda i, c: (body(i), c)[1], 0)

            def start_kv(h):
                k_copy(h).start()
                v_copy(h).start()

            x_copy.start()
            wq_copy.start()
            wr_copy.start()
            loop(0, FFN_AFTER, start_kv)
            wg_copy.start()
            wu_copy.start()
            wd_copy.start()
            loop(FFN_AFTER, HQ, start_kv)
            loop(0, LAST, lambda h: wo_copy(h).start())
            loop(0, len(TAIL), start_wo_tail)

            x_copy.wait()
            x = x_buf[0].astype(F32)
            xc = x - jnp.mean(x, axis=-1, keepdims=True)
            var = jnp.mean(xc * xc, axis=-1, keepdims=True)
            xn = xc / jnp.sqrt(var + LN_EPS)
            xn_b = xn.astype(BF)
            xn_rows = jnp.broadcast_to(xn_b, (ROWS, D))

            wr_copy.wait()
            r = jnp.sum(xn_b.astype(F32) * wr_buf[...].reshape(1, D).astype(F32),
                        axis=-1, keepdims=True)
            r_gate = jax.nn.sigmoid(r)

            wq_copy.wait()
            for h in range(HQ):
                q_scr[h] = lax.dot_general(xn_rows, wq_buf[:, h * DH:(h + 1) * DH], NN,
                                           preferred_element_type=F32).astype(BF)

            def head(h):
                k_copy(h).wait()
                s = lax.dot_general(q_scr[h], k_buf[h], NT, preferred_element_type=F32) * (DH ** -0.5)
                p = jnp.exp(s - jnp.max(s, axis=-1, keepdims=True))
                denom = jnp.sum(p, axis=-1, keepdims=True)
                v_copy(h).wait()
                o = lax.dot_general(p.astype(BF), v_buf[h], NN, preferred_element_type=F32)
                o_scr[h] = (o / denom).astype(BF)

            loop(0, FFN_AFTER, head)

            wg_copy.wait()
            wu_copy.wait()
            g = lax.dot_general(xn_rows, wg_buf[...], NT, preferred_element_type=F32)
            u = lax.dot_general(xn_rows, wu_buf[...], NT, preferred_element_type=F32)
            hid = (g * jax.nn.sigmoid(g) * u).astype(BF)
            wd_copy.wait()
            y = lax.dot_general(hid, wd_buf[...], NN, preferred_element_type=F32)[0:1]
            routed = xn + y * r_gate
            gate = routed * jax.nn.sigmoid(routed)

            loop(FFN_AFTER, HQ, head)

            o_last = o_scr[LAST][0:1, :].astype(F32)
            c_scr[...] = jnp.broadcast_to(o_last, (DH, DH)).T
            acc = jnp.zeros((ROWS, D), F32)
            for h in range(LAST):
                wo_copy(h).wait()
                acc = acc + lax.dot_general(o_scr[h], wo_buf[h * DH:(h + 1) * DH, :], NN,
                                            preferred_element_type=F32)
            part = jnp.zeros((8, D), F32)
            for j, (r0, n) in enumerate(TAIL):
                wo_tail_copy(j).wait()
                w = wo_buf[LAST * DH + r0:LAST * DH + r0 + n, :].astype(F32)
                c = jnp.concatenate([c_scr[r0:r0 + n, :]] * (D // DH), axis=1)
                part = part + (w * c).reshape(n // 8, 8, D).sum(axis=0)
            s_out = acc[0:1] + jnp.sum(part, axis=0, keepdims=True)

            o_ref[0] = (x + s_out * gate).astype(BF)

        pl.run_scoped(
            body,
            pltpu.SemaphoreType.DMA((HQ,)),
            pltpu.SemaphoreType.DMA((HQ,)),
            pltpu.SemaphoreType.DMA((LAST + len(TAIL),)),
            pltpu.SemaphoreType.DMA((6,)),
        )

    hbm = pl.BlockSpec(memory_space=pltpu.HBM)
    return pl.pallas_call(
        kernel,
        out_shape=jax.ShapeDtypeStruct((B, Sq, D), BF),
        in_specs=[hbm] * 9,
        out_specs=pl.BlockSpec(memory_space=pltpu.VMEM),
        scratch_shapes=[
            pltpu.VMEM((B, Sq, D), BF),
            pltpu.VMEM((D,), BF),
            pltpu.VMEM((HQ, W, DH), BF),
            pltpu.VMEM((HQ, W, DH), BF),
            pltpu.VMEM((D, HQ * DH), BF),
            pltpu.VMEM((HQ * DH, D), BF),
            pltpu.VMEM((F, D), BF),
            pltpu.VMEM((F, D), BF),
            pltpu.VMEM((F, D), BF),
            pltpu.VMEM((HQ, ROWS, DH), BF),
            pltpu.VMEM((HQ, ROWS, DH), BF),
            pltpu.VMEM((DH, DH), F32),
        ],
        compiler_params=pltpu.CompilerParams(vmem_limit_bytes=96 * 1024 * 1024),
    )(A_x, A_k_cache, A_v_cache, A_wq, A_wo, B_w_r, B_w_gate.T, B_w_up.T, B_w_down)
```
